```python
import jax
import jax.numpy as jnp

def _softmax(x, axis=-1):
    return jax.nn.softmax(x, axis=axis)
def _gelu(x):
    return jax.nn.gelu(x, approximate=True)
def _silu(x):
    return jax.nn.silu(x)
def _sigmoid(x):
    return jax.nn.sigmoid(x)
def _layernorm(x, axis=-1, eps=1e-5):
    m = jnp.mean(x, axis=axis, keepdims=True)
    v = jnp.var(x, axis=axis, keepdims=True)
    return (x - m) / jnp.sqrt(v + eps)
def _scatter_add(tgt, idx, src, axis=0):
    return tgt.at[idx].add(src)
def _segment_sum(src, seg, n):
    return jax.ops.segment_sum(src, seg, n)
class _Rng:
    def __init__(self, key):
        self._k = key
    def _next(self):
        self._k, sub = jax.random.split(self._k)
        return sub
    def normal(self, shape):
        return jax.random.normal(self._next(), shape, dtype=jnp.bfloat16)
    def randint(self, lo, hi, shape):
        return jax.random.randint(self._next(), shape, lo, hi, dtype=jnp.int32)
    def uniform(self, shape, lo=0.0, hi=1.0):
        return jax.random.uniform(self._next(), shape, jnp.bfloat16, lo, hi)
    def permutation(self, n):
        return jax.random.permutation(self._next(), n)


kernel_name = 'standalone__instancenorm__prompt'

def setup_inputs():
    _rng = _Rng(jax.random.key(int.from_bytes(__import__("os").urandom(4), "little")))
    _w = (lambda a: (lambda t: t.astype(jnp.bfloat16) if jnp.issubdtype(t.dtype, jnp.floating) else t)(jnp.asarray(a)))
    B, C, H, W = 2, 1024, 2048, 32
    return {
        "x": _w((lambda *s: _rng.normal(s) * 0.05)(B, C, H, W)),
        "g": _w((lambda *s: _rng.normal(s) * 0.05)(C) + 1.0),
        "b": _w((lambda *s: _rng.normal(s) * 0.05)(C)),
    }

def reference(x, g, b):
    mu = x.mean(axis=(-2, -1), keepdims=True)
    var = ((x - mu) * (x - mu)).mean(axis=(-2, -1), keepdims=True)
    xhat = (x - mu) / jnp.sqrt(var + 1e-5)
    return xhat * g.reshape(1, -1, 1, 1) + b.reshape(1, -1, 1, 1)
```

```python
import jax
import jax.numpy as jnp
from jax import lax
import jax.experimental.pallas as pl
import jax.experimental.pallas.tpu as pltpu

_EPS = 1e-5


def _build(B, C, H, W, n=4, d=4, R=8, S=16, cols=1024, cpc=4, every=3, delta=1):
    G = (B * C) // (R * S)
    shp = (G, R, S, W, H)
    nc = H // cols
    nh = W // 16
    U = S * nh * nc
    unit_ch = R * 16 * cols // (W * H)
    Q = n + 1
    PS = 2 * n * U
    total = (G // n) * PS
    nchunk = n * R * S // cpc
    inv_n = 1.0 / (H * W)

    def kernel(x_hbm, g_ref, b_ref, o_hbm, buf, gb_v, gb_s, sems, gsem):
        def wsl(u):
            j = u // (nh * nc)
            h = (u // nc) % nh
            c = u % nc
            return (slice(None), j, pl.ds(pl.multiple_of(h * 16, 16), 16),
                    pl.ds(pl.multiple_of(c * cols, 128), cols))

        def rd(g, u, ss):
            ch = u * unit_ch
            r = ch // S
            j = ch % S
            return pltpu.make_async_copy(
                x_hbm.at[g, r, pl.ds(j, unit_ch)],
                buf.at[g % Q, r, pl.ds(j, unit_ch)], sems.at[ss])

        def wr(g, u, ss):
            return pltpu.make_async_copy(
                buf.at[(g % Q,) + wsl(u)], o_hbm.at[(g,) + wsl(u)], sems.at[ss])

        def decode(s):
            p = s // PS
            w = s % PS
            isw = w >= n * U
            w2 = jnp.where(isw, w - n * U, w)
            return isw, p * n + w2 // U, w2 % U

        def start(s):
            isw, g, u = decode(s)

            @pl.when(jnp.logical_not(isw))
            def _():
                rd(g, u, s % d).start()

            @pl.when(isw)
            def _():
                wr(g, u, s % d).start()

        def wait(s):
            isw, g, u = decode(s)

            @pl.when(jnp.logical_not(isw))
            def _():
                rd(g, u, s % d).wait()

            @pl.when(isw)
            def _():
                wr(g, u, s % d).wait()

        for s in range(d):
            rd(0, s, s).start()
        gb_v[0] = g_ref[...].astype(jnp.float32)
        gb_v[1] = b_ref[...].astype(jnp.float32)
        cp = pltpu.make_async_copy(gb_v, gb_s, gsem)
        cp.start()
        cp.wait()

        def compute(p, c):
            ch0 = c * cpc
            g = p * n + ch0 // (R * S)
            r = (ch0 // S) % R
            j0 = ch0 % S
            slot = g % Q
            cg = (g * R * S + r * S + j0) % C
            refs = [buf.at[slot, r, j0 + t] for t in range(cpc)]
            mus = [jnp.sum(rf[...].astype(jnp.float32), keepdims=True) * inv_n
                   for rf in refs]
            vs = []
            for rf, mu in zip(refs, mus):
                dx = rf[...].astype(jnp.float32) - mu
                vs.append(jnp.sum(dx * dx, keepdims=True) * inv_n)
            for t, (rf, mu, var) in enumerate(zip(refs, mus, vs)):
                gs = gb_s[0, (cg + t) // 128, (cg + t) % 128]
                bs = gb_s[1, (cg + t) // 128, (cg + t) % 128]
                sc = lax.rsqrt(var + _EPS) * gs
                sh = bs - mu * sc
                rf[...] = (rf[...].astype(jnp.float32) * sc + sh).astype(jnp.bfloat16)

        def body(s, carry):
            wait(s)

            @pl.when(s + d < total)
            def _():
                start(s + d)

            p = s // PS
            w = s % PS - delta
            c = w // every

            @pl.when(jnp.logical_and(jnp.logical_and(w >= 0, w % every == 0), c < nchunk))
            def _():
                compute(p, c)

            return carry

        lax.fori_loop(0, total, body, 0)

    scratch = [
        pltpu.VMEM((Q, R, S, W, H), jnp.bfloat16),
        pltpu.VMEM((2, 8, 128), jnp.float32),
        pltpu.SMEM((2, 8, 128), jnp.float32),
        pltpu.SemaphoreType.DMA((d,)),
        pltpu.SemaphoreType.DMA(()),
    ]
    return kernel, shp, scratch


@jax.jit
def pallas_standalone__instancenorm__prompt_kernel(
    x: jax.Array,
    g: jax.Array,
    b: jax.Array,
):
    B, C, H, W = x.shape
    kernel, shp, scratch = _build(B, C, H, W)
    xt = jnp.transpose(x, (0, 1, 3, 2)).reshape(shp)
    o = pl.pallas_call(
        kernel,
        in_specs=[
            pl.BlockSpec(memory_space=pl.ANY),
            pl.BlockSpec(memory_space=pltpu.VMEM),
            pl.BlockSpec(memory_space=pltpu.VMEM),
        ],
        out_specs=pl.BlockSpec(memory_space=pl.ANY),
        out_shape=jax.ShapeDtypeStruct(shp, x.dtype),
        scratch_shapes=scratch,
        compiler_params=pltpu.CompilerParams(vmem_limit_bytes=120 * 1024 * 1024),
    )(xt, g.reshape(8, 128), b.reshape(8, 128))
    return jnp.transpose(o.reshape(B, C, W, H), (0, 1, 3, 2))
```

```python
import jax
import jax.numpy as jnp
from jax import lax
import jax.experimental.pallas as pl
import jax.experimental.pallas.tpu as pltpu

_EPS = 1e-5

_R, _S = 8, 16
_PHASES = (4, 4, 4, 4)
_MC = 4
_PIECE = (16, 1024)
_NGR, _NGW = 8, 3
_LEAD_R = 1
_RING = 8


def _shr(a, v):
    if isinstance(a, int):
        return a // v
    return lax.shift_right_logical(a, jnp.int32(v.bit_length() - 1))


def _make_kernel(C, W, H):
    rows, cols = _PIECE
    nh, nc = W // rows, H // cols
    upw = _MC * nh * nc // _R
    spg = _R * _S // _MC
    inv_n = 1.0 / (W * H)

    def kernel(x_hbm, g_hbm, b_hbm, o_hbm, buf, gb_raw, gb_vmem, gb, rsem, wsem, gsem):
        buf5 = buf.reshape(max(_PHASES), _R, _S, W, H)

        def rd_start(c0, i):
            n = 0
            for t in range(_MC):
                for h in range(nh):
                    for c in range(nc):
                        sl = (pl.ds(h * rows, rows), pl.ds(c * cols, cols))
                        pltpu.make_async_copy(
                            x_hbm.at[(c0 + i * _MC + t,) + sl],
                            buf.at[(i * _MC + t,) + sl],
                            rsem.at[i & (_RING - 1)],
                        ).start(priority=n % 2)
                        n += 1

        def rd_wait(i):
            dst = buf.at[pl.ds(i * _MC, _MC)]
            pltpu.make_async_copy(dst, dst, rsem.at[i & (_RING - 1)]).wait()

        def wr_copies(g0, i):
            gl = _shr(i, spg)
            copies = []
            for m in range(upw):
                u = (i & (spg - 1)) * upw + m
                r0 = (_shr(u, nc) & (nh - 1)) * rows
                c0 = (u & (nc - 1)) * cols
                if not isinstance(u, int):
                    r0, c0 = pl.multiple_of(r0, rows), pl.multiple_of(c0, cols)
                sl = (slice(None), _shr(u, nh * nc), pl.ds(r0, rows), pl.ds(c0, cols))
                copies.append(pltpu.make_async_copy(
                    buf5.at[(gl,) + sl], o_hbm.at[(g0 + gl,) + sl],
                    wsem.at[i & (_RING - 1)]))
            return copies

        def wr_start(g0, i):
            for cp in wr_copies(g0, i):
                cp.start()

        def wr_wait(g0, i):
            for cp in wr_copies(g0, i):
                cp.wait()

        def normalise(c0, i):
            refs = [buf.at[i * _MC + t] for t in range(_MC)]
            means = [jnp.sum(r[...].astype(jnp.float32), keepdims=True) * inv_n
                     for r in refs]
            variances = []
            for r, mu in zip(refs, means):
                d = r[...].astype(jnp.float32) - mu
                variances.append(jnp.sum(d * d, keepdims=True) * inv_n)
            for t, (r, mu, var) in enumerate(zip(refs, means, variances)):
                ch = (c0 + i * _MC + t) & (C - 1)
                row, col = _shr(ch, 128), ch & 127
                scale = lax.rsqrt(var + _EPS) * gb[0, row, col]
                shift = gb[1, row, col] - mu * scale
                r[...] = (r[...].astype(jnp.float32) * scale + shift).astype(r.dtype)

        cp_g = pltpu.make_async_copy(g_hbm, gb_raw.at[0], gsem.at[0])
        cp_b = pltpu.make_async_copy(b_hbm, gb_raw.at[1], gsem.at[1])
        rd_start(0, 0)
        cp_g.start()
        cp_b.start()
        for i in range(1, _NGR):
            rd_start(0, i)
        cp_g.wait()
        cp_b.wait()
        gb_vmem[...] = gb_raw[...].astype(jnp.float32)
        cp_s = pltpu.make_async_copy(gb_vmem, gb, gsem.at[0])
        cp_s.start()
        cp_s.wait()

        g0 = 0
        for p, n in enumerate(_PHASES):
            c0 = g0 * _R * _S
            ns = n * spg
            half = ns // 2
            more = p + 1 < len(_PHASES)

            def read_step(i, tail):
                rd_wait(i)
                if tail:
                    @pl.when(i >= ns - _NGW)
                    def _():
                        wr_start(g0, i - (ns - _NGW))
                else:
                    rd_start(c0, i + _NGR)

                @pl.when((i & 1) == 0)
                def _():
                    normalise(c0, _shr(i, 2))

            lax.fori_loop(0, ns - _NGR, lambda i, _: read_step(i, False), None)
            lax.fori_loop(ns - _NGR, ns, lambda i, _: read_step(i, True), None)

            def write_step(i, compute):
                wr_wait(g0, i)
                wr_start(g0, i + _NGW)
                if compute:
                    normalise(c0, half + i)

            lax.fori_loop(0, half, lambda i, _: write_step(i, True), None)
            lax.fori_loop(half, ns - _NGW, lambda i, _: write_step(i, False), None)
            c1 = (g0 + n) * _R * _S
            for i in range(ns - _NGW, ns):
                wr_wait(g0, i)
                if more and i >= ns - _LEAD_R:
                    rd_start(c1, i - (ns - _LEAD_R))
            if more:
                for i in range(_LEAD_R, _NGR):
                    rd_start(c1, i)
            g0 += n

    return kernel


@jax.jit
def pallas_standalone__instancenorm__prompt_kernel(
    x: jax.Array,
    g: jax.Array,
    b: jax.Array,
):
    B, C, H, W = x.shape
    G = B * C // (_R * _S)
    xt = jnp.transpose(x, (0, 1, 3, 2)).reshape(B * C, W, H)
    o = pl.pallas_call(
        _make_kernel(C, W, H),
        in_specs=[pl.BlockSpec(memory_space=pl.ANY)] * 3,
        out_specs=pl.BlockSpec(memory_space=pl.ANY),
        out_shape=jax.ShapeDtypeStruct((G, _R, _S, W, H), x.dtype),
        scratch_shapes=[
            pltpu.VMEM((max(_PHASES) * _R * _S, W, H), x.dtype),
            pltpu.VMEM((2, C // 128, 128), g.dtype),
            pltpu.VMEM((2, C // 128, 128), jnp.float32),
            pltpu.SMEM((2, C // 128, 128), jnp.float32),
            pltpu.SemaphoreType.DMA((_RING,)),
            pltpu.SemaphoreType.DMA((_RING,)),
            pltpu.SemaphoreType.DMA((2,)),
        ],
        compiler_params=pltpu.CompilerParams(vmem_limit_bytes=120 * 1024 * 1024),
    )(xt, g.reshape(C // 128, 128), b.reshape(C // 128, 128))
    return jnp.transpose(o.reshape(B, C, W, H), (0, 1, 3, 2))
```

```python
import jax
import jax.numpy as jnp
from jax import lax
import jax.experimental.pallas as pl
import jax.experimental.pallas.tpu as pltpu

_EPS = 1e-5

_R, _S = 8, 16
_PHASES = (4, 4, 4, 4)
_MC = 4
_PIECE = (16, 1024)
_NGR, _NGW = 8, 3
_LEAD_R = 1
_RING = 8


def _shr(a, v):
    if isinstance(a, int):
        return a // v
    return lax.shift_right_logical(a, jnp.int32(v.bit_length() - 1))


def _make_kernel(C, W, H):
    rows, cols = _PIECE
    nh, nc = W // rows, H // cols
    upw = _MC * nh * nc // _R
    spg = _R * _S // _MC
    inv_n = 1.0 / (W * H)

    def kernel(x_hbm, g_hbm, b_hbm, o_hbm, buf, gb_raw, gb_vmem, gb, rsem, wsem, gsem):
        buf5 = buf.reshape(max(_PHASES), _R, _S, W, H)

        def pieces(i):
            out = []
            for m in range(upw):
                u = (i & (spg - 1)) * upw + m
                r0 = (_shr(u, nc) & (nh - 1)) * rows
                c0 = (u & (nc - 1)) * cols
                if not isinstance(u, int):
                    r0, c0 = pl.multiple_of(r0, rows), pl.multiple_of(c0, cols)
                out.append((_shr(u, nh * nc), (pl.ds(r0, rows), pl.ds(c0, cols))))
            return out

        def rd_start(c0, i):
            base = _shr(i, spg) * (_R * _S)
            for j, win in pieces(i):
                for r in range(_R):
                    inst = base + r * _S + j
                    pltpu.make_async_copy(
                        x_hbm.at[(c0 + inst,) + win], buf.at[(inst,) + win],
                        rsem.at[i & (_RING - 1)],
                    ).start(priority=r % 2)

        def rd_wait(i):
            dst = buf.at[pl.ds(i * _MC, _MC)]
            pltpu.make_async_copy(dst, dst, rsem.at[i & (_RING - 1)]).wait()

        def wr_copies(g0, i):
            gl = _shr(i, spg)
            return [
                pltpu.make_async_copy(
                    buf5.at[(gl, slice(None), j) + win],
                    o_hbm.at[(g0 + gl, slice(None), j) + win],
                    wsem.at[i & (_RING - 1)])
                for j, win in pieces(i)]

        def wr_start(g0, i):
            for cp in wr_copies(g0, i):
                cp.start()

        def wr_wait(g0, i):
            for cp in wr_copies(g0, i):
                cp.wait()

        def normalise(c0, i):
            refs = [buf.at[i * _MC + t] for t in range(_MC)]
            means = [jnp.sum(r[...].astype(jnp.float32), keepdims=True) * inv_n
                     for r in refs]
            variances = []
            for r, mu in zip(refs, means):
                d = r[...].astype(jnp.float32) - mu
                variances.append(jnp.sum(d * d, keepdims=True) * inv_n)
            for t, (r, mu, var) in enumerate(zip(refs, means, variances)):
                ch = (c0 + i * _MC + t) & (C - 1)
                row, col = _shr(ch, 128), ch & 127
                scale = lax.rsqrt(var + _EPS) * gb[0, row, col]
                shift = gb[1, row, col] - mu * scale
                r[...] = (r[...].astype(jnp.float32) * scale + shift).astype(r.dtype)

        cp_g = pltpu.make_async_copy(g_hbm, gb_raw.at[0], gsem.at[0])
        cp_b = pltpu.make_async_copy(b_hbm, gb_raw.at[1], gsem.at[1])
        rd_start(0, 0)
        cp_g.start()
        cp_b.start()
        for i in range(1, _NGR):
            rd_start(0, i)
        cp_g.wait()
        cp_b.wait()
        gb_vmem[...] = gb_raw[...].astype(jnp.float32)
        cp_s = pltpu.make_async_copy(gb_vmem, gb, gsem.at[0])
        cp_s.start()
        cp_s.wait()

        g0 = 0
        for p, n in enumerate(_PHASES):
            c0 = g0 * _R * _S
            ns = n * spg
            n_rd = (ns - spg) // 2
            n_wr = ns - n_rd
            assert all((k + 1) * spg <= n_rd or
                       (k + 1) * spg - n_rd < k * spg - _NGW for k in range(n))
            more = p + 1 < len(_PHASES)

            def read_step(i, tail):
                rd_wait(i)
                if tail:
                    @pl.when(i >= ns - _NGW)
                    def _():
                        wr_start(g0, i - (ns - _NGW))
                else:
                    rd_start(c0, i + _NGR)

                @pl.when(jnp.logical_and(i >= spg, (i & 1) == 0))
                def _():
                    normalise(c0, _shr(i - spg, 2))

            lax.fori_loop(0, ns - _NGR, lambda i, _: read_step(i, False), None)
            lax.fori_loop(ns - _NGR, ns, lambda i, _: read_step(i, True), None)

            def write_step(i, compute):
                wr_wait(g0, i)
                wr_start(g0, i + _NGW)
                if compute:
                    normalise(c0, n_rd + i)

            lax.fori_loop(0, n_wr, lambda i, _: write_step(i, True), None)
            lax.fori_loop(n_wr, ns - _NGW, lambda i, _: write_step(i, False), None)
            c1 = (g0 + n) * _R * _S
            for i in range(ns - _NGW, ns):
                wr_wait(g0, i)
                if more and i >= ns - _LEAD_R:
                    rd_start(c1, i - (ns - _LEAD_R))
            if more:
                for i in range(_LEAD_R, _NGR):
                    rd_start(c1, i)
            g0 += n

    return kernel


@jax.jit
def pallas_standalone__instancenorm__prompt_kernel(
    x: jax.Array,
    g: jax.Array,
    b: jax.Array,
):
    B, C, H, W = x.shape
    G = B * C // (_R * _S)
    xt = jnp.transpose(x, (0, 1, 3, 2)).reshape(B * C, W, H)
    o = pl.pallas_call(
        _make_kernel(C, W, H),
        in_specs=[pl.BlockSpec(memory_space=pl.ANY)] * 3,
        out_specs=pl.BlockSpec(memory_space=pl.ANY),
        out_shape=jax.ShapeDtypeStruct((G, _R, _S, W, H), x.dtype),
        scratch_shapes=[
            pltpu.VMEM((max(_PHASES) * _R * _S, W, H), x.dtype),
            pltpu.VMEM((2, C // 128, 128), g.dtype),
            pltpu.VMEM((2, C // 128, 128), jnp.float32),
            pltpu.SMEM((2, C // 128, 128), jnp.float32),
            pltpu.SemaphoreType.DMA((_RING,)),
            pltpu.SemaphoreType.DMA((_RING,)),
            pltpu.SemaphoreType.DMA((2,)),
        ],
        compiler_params=pltpu.CompilerParams(vmem_limit_bytes=120 * 1024 * 1024),
    )(xt, g.reshape(C // 128, 128), b.reshape(C // 128, 128))
    return jnp.transpose(o.reshape(B, C, W, H), (0, 1, 3, 2))
```
